```python
import os as _os
_os.environ.setdefault("JAX_PLATFORMS", "cpu")
import jax
import jax.numpy as jnp

def _softmax(x, axis=-1):
    return jax.nn.softmax(x, axis=axis)
def _gelu(x):
    return jax.nn.gelu(x, approximate=True)
def _silu(x):
    return jax.nn.silu(x)
def _sigmoid(x):
    return jax.nn.sigmoid(x)
def _layernorm(x, axis=-1, eps=1e-5):
    m = jnp.mean(x, axis=axis, keepdims=True)
    v = jnp.var(x, axis=axis, keepdims=True)
    return (x - m) / jnp.sqrt(v + eps)
def _scatter_add(tgt, idx, src, axis=0):
    return tgt.at[idx].add(src)
def _segment_sum(src, seg, n):
    return jax.ops.segment_sum(src, seg, n)
class _Rng:
    def __init__(self, key):
        self._k = key
    def _next(self):
        self._k, sub = jax.random.split(self._k)
        return sub
    def normal(self, shape):
        return jax.random.normal(self._next(), shape, dtype=jnp.bfloat16)
    def randint(self, lo, hi, shape):
        return jax.random.randint(self._next(), shape, lo, hi, dtype=jnp.int32)
    def uniform(self, shape, lo=0.0, hi=1.0):
        return jax.random.uniform(self._next(), shape, jnp.bfloat16, lo, hi)
    def permutation(self, n):
        return jax.random.permutation(self._next(), n)


kernel_name = 'standalone__gqa_block_cached__near_ridge'

def setup_inputs():
    _rng = _Rng(jax.random.key(int.from_bytes(__import__("os").urandom(4), "little")))
    _w = (lambda a: (lambda t: t.astype(jnp.bfloat16) if jnp.issubdtype(t.dtype, jnp.floating) else t)(jnp.asarray(a)))
    B, Sq, D = 8, 64, 512
    Hq, Hkv, Sk, Dh = 32, 8, 64, 128
    assert Hq % Hkv == 0, (Hq, Hkv)
    return {
        "x": _w((lambda *s: _rng.normal(s) * 0.8)(B, Sq, D)),
        "k_cache": _w((lambda *s: _rng.normal(s) * 0.8)(B, Hkv, Sk, Dh)),
        "v_cache": _w((lambda *s: _rng.normal(s) * 0.05)(B, Hkv, Sk, Dh)),
        "wq": _w((lambda *s: _rng.normal(s) * 0.8)(D, Hq * Dh) * (D ** -0.5)),
        "wo": _w((lambda *s: _rng.normal(s) * 0.05)(Hq * Dh, D) * ((Hq * Dh) ** -0.5)),
    }

def reference(x, k_cache, v_cache, wq, wo):
    B, Sq, D = x.shape
    Hq, Dh = 32, 128
    Hkv = k_cache.shape[1]
    rep = Hq // Hkv
    q = (lambda x, *d: x.transpose(*d))((x @ wq).reshape(B, Sq, Hq, Dh), 0, 2, 1, 3)
    k = jnp.repeat(k_cache, rep, axis=1)
    v = jnp.repeat(v_cache, rep, axis=1)
    scores = jnp.einsum("bhqd,bhkd->bhqk", q, k) * (Dh ** -0.5)
    p = _softmax(scores, axis=-1)
    o = jnp.einsum("bhqk,bhkd->bhqd", p, v)
    return (lambda x, *d: x.transpose(*d))(o, 0, 2, 1, 3).reshape(B, Sq, Hq * Dh) @ wo
```

```python
import jax
import jax.numpy as jnp
import jax.experimental.pallas as pl
import jax.experimental.pallas.tpu as pltpu

B, SQ, D = 8, 64, 512
HQ, HKV, SK, DH = 32, 8, 64, 128
REP = HQ // HKV
GW = REP * DH


def _kernel(x_ref, wq_ref, k_ref, v_ref, wo_ref, o_ref, acc_ref):
    g = pl.program_id(0)
    scale = DH ** -0.5

    @pl.when(g == 0)
    def _():
        acc_ref[...] = jnp.zeros_like(acc_ref)

    q = jnp.dot(x_ref[...], wq_ref[...], preferred_element_type=jnp.float32)
    q = q.astype(jnp.bfloat16)
    outs = []
    for b in range(B):
        qb = q[b * SQ:(b + 1) * SQ]
        qs = jnp.concatenate([qb[:, r * DH:(r + 1) * DH] for r in range(REP)], axis=0)
        s = jax.lax.dot_general(qs, k_ref[b, 0], (((1,), (1,)), ((), ())),
                                preferred_element_type=jnp.float32) * scale
        m = jnp.max(s, axis=-1, keepdims=True)
        p = jnp.exp(s - m)
        l = jnp.sum(p, axis=-1, keepdims=True)
        o = jnp.dot(p.astype(jnp.bfloat16), v_ref[b, 0], preferred_element_type=jnp.float32)
        o = o / l
        ob = jnp.concatenate([o[r * SQ:(r + 1) * SQ] for r in range(REP)], axis=1)
        outs.append(ob.astype(jnp.bfloat16))
    og = jnp.concatenate(outs, axis=0)
    acc_ref[...] += jnp.dot(og, wo_ref[...], preferred_element_type=jnp.float32)

    @pl.when(g == HKV - 1)
    def _():
        o_ref[...] = acc_ref[...].astype(o_ref.dtype)


@jax.jit
def pallas_standalone__gqa_block_cached__near_ridge_kernel(x, k_cache, v_cache, wq, wo):
    x2 = x.reshape(B * SQ, D)
    out = pl.pallas_call(
        _kernel,
        grid=(HKV,),
        in_specs=[
            pl.BlockSpec((B * SQ, D), lambda g: (0, 0)),
            pl.BlockSpec((D, GW), lambda g: (0, g)),
            pl.BlockSpec((B, 1, SK, DH), lambda g: (0, g, 0, 0)),
            pl.BlockSpec((B, 1, SK, DH), lambda g: (0, g, 0, 0)),
            pl.BlockSpec((GW, D), lambda g: (g, 0)),
        ],
        out_specs=pl.BlockSpec((B * SQ, D), lambda g: (0, 0)),
        out_shape=jax.ShapeDtypeStruct((B * SQ, D), jnp.bfloat16),
        scratch_shapes=[pltpu.VMEM((B * SQ, D), jnp.float32)],
        compiler_params=pltpu.CompilerParams(
            dimension_semantics=("arbitrary",),
            vmem_limit_bytes=64 * 1024 * 1024,
        ),
    )(x2, wq, k_cache, v_cache, wo)
    return out.reshape(B, SQ, D)
```

```python
import jax
import jax.numpy as jnp
import jax.experimental.pallas as pl
import jax.experimental.pallas.tpu as pltpu

B, SQ, D = 8, 64, 512
HQ, HKV, SK, DH = 32, 8, 64, 128
REP = HQ // HKV
GW = REP * DH
M = B * SQ
LOG2E = 1.4426950408889634

NKC = 2
NOC = 4

PLAN = (
    (('A', 1),),
    (('A', 2),),
    (('B', 0), ('B', 1), ('A', 3)),
    (('B', 2), ('A', 4), ('C', 0), ('B', 3), ('A', 5), ('C', 1)),
    (('B', 4), ('A', 6), ('C', 2), ('B', 5), ('A', 7), ('C', 3), ('B', 6), ('C', 4), ('B', 7), ('C', 5),
     ('C', 6), ('C', 7)),
)


def _check_plan(plan):
    pos = {('A', 0): -1}
    for i, it in enumerate([it for reg in plan for it in reg]):
        assert it not in pos, it
        pos[it] = i
    for g in range(HKV):
        assert pos[('A', g)] < pos[('B', g)] < pos[('C', g)], g
    for g in range(1, HKV):
        assert pos[('C', g - 1)] < pos[('C', g)], g


_check_plan(PLAN)
NSEM = 2 * NKC + (HKV - 1) + 3 * HKV + NOC


def _attention(q_src, k_ref, v_ref, o_dst, g, b):
    c = (DH ** -0.5) * LOG2E
    qs = jnp.concatenate([q_src[b * SQ:(b + 1) * SQ, r * DH:(r + 1) * DH] for r in range(REP)], axis=0)
    s = jax.lax.dot_general(qs, k_ref[b, g], (((1,), (1,)), ((), ())),
                            preferred_element_type=jnp.float32)
    m = jnp.max(s, axis=-1, keepdims=True)
    p = jnp.exp2((s - m) * c)
    l = jnp.sum(p, axis=-1, keepdims=True)
    r0 = pl.reciprocal(l, approx=True)
    rl = r0 * (2.0 - l * r0)
    o = jnp.dot(p.astype(jnp.bfloat16), v_ref[b, g], preferred_element_type=jnp.float32)
    o = (o * rl).astype(jnp.bfloat16)
    for r in range(REP):
        o_dst[b * SQ:(b + 1) * SQ, r * DH:(r + 1) * DH] = o[r * SQ:(r + 1) * SQ]


def _kernel(x_hbm, k_hbm, v_hbm, wq_hbm, wo_hbm, out_hbm, *scr):
    x_v, k_v, v_v, wq_v, wo_v, acc_ref, out_v, qacc, sems = scr[:9]
    q_bufs = scr[9:9 + HKV]
    o_bufs = scr[9 + HKV:9 + 2 * HKV]
    KC = D // NKC
    OC = D // NOC
    f32 = jnp.float32

    n_used = [0]

    def sem():
        n_used[0] += 1
        return sems.at[n_used[0] - 1]

    cx = [pltpu.make_async_copy(x_hbm.at[:, pl.ds(i * KC, KC)], x_v.at[:, pl.ds(i * KC, KC)], sem())
          for i in range(NKC)]
    cwq0 = [pltpu.make_async_copy(wq_hbm.at[pl.ds(i * KC, KC), pl.ds(0, GW)], wq_v.at[0, pl.ds(i * KC, KC), :], sem())
            for i in range(NKC)]
    cwq = [None] + [pltpu.make_async_copy(wq_hbm.at[:, pl.ds(g * GW, GW)], wq_v.at[g], sem())
                    for g in range(1, HKV)]
    ck = [pltpu.make_async_copy(k_hbm.at[:, pl.ds(g, 1)], k_v.at[:, pl.ds(g, 1)], sem()) for g in range(HKV)]
    cv = [pltpu.make_async_copy(v_hbm.at[:, pl.ds(g, 1)], v_v.at[:, pl.ds(g, 1)], sem()) for g in range(HKV)]
    cwo = [pltpu.make_async_copy(wo_hbm.at[pl.ds(g * GW, GW), :], wo_v.at[g], sem()) for g in range(HKV)]
    cout = [pltpu.make_async_copy(out_v.at[:, pl.ds(i * OC, OC)], out_hbm.at[:, pl.ds(i * OC, OC)], sem())
            for i in range(NOC)]
    assert n_used[0] == NSEM

    def copies_for(item):
        kind, g = item
        return {'A': (cwq[g],), 'B': (ck[g], cv[g]), 'C': (cwo[g],)}[kind]

    for i in range(NKC):
        cx[i].start()
        cwq0[i].start()
    for reg in PLAN:
        for it in reg:
            for cp in copies_for(it):
                cp.start()

    for i in range(NKC):
        cx[i].wait()
        cwq0[i].wait()
        part = jnp.dot(x_v[:, pl.ds(i * KC, KC)], wq_v[0, pl.ds(i * KC, KC), :], preferred_element_type=f32)
        if i == 0:
            qacc[...] = part
        elif i < NKC - 1:
            qacc[...] += part
        else:
            q_bufs[0][...] = (qacc[...] + part).astype(jnp.bfloat16)

    for reg in PLAN:
        for it in reg:
            for cp in copies_for(it):
                cp.wait()
        for kind, g in reg:
            if kind == 'A':
                q_bufs[g][...] = jnp.dot(x_v[...], wq_v[g], preferred_element_type=f32).astype(jnp.bfloat16)
            elif kind == 'B':
                for b in range(B):
                    _attention(q_bufs[g], k_v, v_v, o_bufs[g], g, b)
            elif g == 0:
                acc_ref[...] = jnp.dot(o_bufs[g][...], wo_v[g], preferred_element_type=f32)
            elif g < HKV - 1:
                acc_ref[...] += jnp.dot(o_bufs[g][...], wo_v[g], preferred_element_type=f32)
            else:
                for i in range(NOC):
                    cols = pl.ds(i * OC, OC)
                    out_v[:, cols] = (acc_ref[:, cols]
                                      + jnp.dot(o_bufs[g][...], wo_v[g, :, cols], preferred_element_type=f32)
                                      ).astype(out_v.dtype)
                    cout[i].start()
    for cp in cout:
        cp.wait()


@jax.jit
def pallas_standalone__gqa_block_cached__near_ridge_kernel(
    x: jax.Array,
    k_cache: jax.Array,
    v_cache: jax.Array,
    wq: jax.Array,
    wo: jax.Array,
):
    bf16, f32 = jnp.bfloat16, jnp.float32
    out = pl.pallas_call(
        _kernel,
        in_specs=[pl.BlockSpec(memory_space=pl.ANY)] * 5,
        out_specs=pl.BlockSpec(memory_space=pl.ANY),
        out_shape=jax.ShapeDtypeStruct((M, D), bf16),
        scratch_shapes=[
            pltpu.VMEM((M, D), bf16),
            pltpu.VMEM((B, HKV, SK, DH), bf16),
            pltpu.VMEM((B, HKV, SK, DH), bf16),
            pltpu.VMEM((HKV, D, GW), bf16),
            pltpu.VMEM((HKV, GW, D), bf16),
            pltpu.VMEM((M, D), f32),
            pltpu.VMEM((M, D), bf16),
            pltpu.VMEM((M, GW), f32),
            pltpu.SemaphoreType.DMA((NSEM,)),
        ] + [pltpu.VMEM((M, GW), bf16) for _ in range(2 * HKV)],
        compiler_params=pltpu.CompilerParams(vmem_limit_bytes=100 * 1024 * 1024),
    )(x.reshape(M, D), k_cache, v_cache, wq, wo)
    return out.reshape(B, SQ, D)
```

```python
import jax
import jax.numpy as jnp
import jax.experimental.pallas as pl
import jax.experimental.pallas.tpu as pltpu

B, SQ, D = 8, 64, 512
HQ, HKV, SK, DH = 32, 8, 64, 128
REP = HQ // HKV
GW = REP * DH
M = B * SQ
LOG2E = 1.4426950408889634

NKC = 4
NOC = 4


def _fused_chunks(groups, first):
    return tuple(tuple(('Ak', g, i) for g in groups) for i in range(first, NKC))


PLAN = (
    (('Ak', 0, 0),),
    (('Ak', 1, 0), ('Ak', 2, 0)),
) + _fused_chunks((0, 1, 2), 1) + (
    (('B', 0), ('B', 1), ('A', 3)),
    (('B', 2), ('A', 4), ('C', 0), ('B', 3), ('A', 5), ('C', 1)),
    (('B', 4), ('A', 6), ('B', 5), ('C', 2), ('A', 7), ('B', 6), ('C', 3), ('B', 7), ('C', 4), ('C', 5),
     ('C', 6), ('C', 7)),
)
ITEMS = tuple(it for reg in PLAN for it in reg)
CHUNKED = tuple(sorted({it[1] for it in ITEMS if it[0] == 'Ak'}))
NSEM = len(PLAN) + 1


def _check_plan():
    first, last, chunks = {}, {}, {}
    for i, it in enumerate(ITEMS):
        key = ('A' if it[0] == 'Ak' else it[0], it[1])
        first.setdefault(key, i)
        last[key] = i
        if it[0] == 'Ak':
            chunks.setdefault(it[1], []).append(it[2])
        else:
            assert ITEMS.count(it) == 1, it
    assert 0 in CHUNKED
    for g, lst in chunks.items():
        assert lst == list(range(NKC)), (g, lst)
    for g in range(HKV):
        assert last[('A', g)] < first[('B', g)] < first[('C', g)], g
    for g in range(1, HKV):
        assert last[('C', g - 1)] < first[('C', g)], g
    for it in ITEMS:
        if it[0] == 'Ak' and it[1] != 0:
            assert ITEMS.index(('Ak', 0, it[2])) <= ITEMS.index(it), it


_check_plan()


def _attention(q_src, k_ref, v_ref, o_dst, g, b):
    c = (DH ** -0.5) * LOG2E
    qs = jnp.concatenate([q_src[b * SQ:(b + 1) * SQ, r * DH:(r + 1) * DH] for r in range(REP)], axis=0)
    s = jax.lax.dot_general(qs, k_ref[b, g], (((1,), (1,)), ((), ())),
                            preferred_element_type=jnp.float32)
    m = jnp.max(s, axis=-1, keepdims=True)
    p = jnp.exp2((s - m) * c)
    l = jnp.sum(p, axis=-1, keepdims=True)
    r0 = pl.reciprocal(l, approx=True)
    rl = r0 * (2.0 - l * r0)
    o = jnp.dot(p.astype(jnp.bfloat16), v_ref[b, g], preferred_element_type=jnp.float32)
    o = (o * rl).astype(jnp.bfloat16)
    for r in range(REP):
        o_dst[b * SQ:(b + 1) * SQ, r * DH:(r + 1) * DH] = o[r * SQ:(r + 1) * SQ]


def _kernel(x_hbm, k_hbm, v_hbm, wq_hbm, wo_hbm, out_hbm, *scr):
    x_v, k_v, v_v, wq_v, wo_v, acc_ref, out_v, sems = scr[:8]
    q_bufs = scr[8:8 + HKV]
    o_bufs = scr[8 + HKV:8 + 2 * HKV]
    qaccs = dict(zip(CHUNKED, scr[8 + 2 * HKV:]))
    KC = D // NKC
    OC = D // NOC
    f32 = jnp.float32

    copies = {}
    for ri, reg in enumerate(PLAN):
        sem = sems.at[ri]
        for it in reg:
            kind, g = it[0], it[1]
            if kind == 'Ak':
                rows = pl.ds(it[2] * KC, KC)
                cs = []
                if g == 0:
                    cs.append(pltpu.make_async_copy(x_hbm.at[:, rows], x_v.at[:, rows], sem))
                cs.append(pltpu.make_async_copy(wq_hbm.at[rows, pl.ds(g * GW, GW)], wq_v.at[g, rows, :], sem))
            elif kind == 'A':
                cs = [pltpu.make_async_copy(wq_hbm.at[:, pl.ds(g * GW, GW)], wq_v.at[g], sem)]
            elif kind == 'B':
                cs = [pltpu.make_async_copy(k_hbm.at[:, pl.ds(g, 1)], k_v.at[:, pl.ds(g, 1)], sem),
                      pltpu.make_async_copy(v_hbm.at[:, pl.ds(g, 1)], v_v.at[:, pl.ds(g, 1)], sem)]
            else:
                cs = [pltpu.make_async_copy(wo_hbm.at[pl.ds(g * GW, GW), :], wo_v.at[g], sem)]
            copies[it] = cs
    cout = [pltpu.make_async_copy(out_v.at[:, pl.ds(i * OC, OC)], out_hbm.at[:, pl.ds(i * OC, OC)],
                                  sems.at[len(PLAN)]) for i in range(NOC)]

    for it in ITEMS:
        for cp in copies[it]:
            cp.start()

    for reg in PLAN:
        for it in reg:
            for cp in copies[it]:
                cp.wait()
        for it in reg:
            kind, g = it[0], it[1]
            if kind == 'Ak':
                i = it[2]
                rows = pl.ds(i * KC, KC)
                part = jnp.dot(x_v[:, rows], wq_v[g, rows, :], preferred_element_type=f32)
                if i == 0:
                    qaccs[g][...] = part
                elif i < NKC - 1:
                    qaccs[g][...] += part
                else:
                    q_bufs[g][...] = (qaccs[g][...] + part).astype(jnp.bfloat16)
            elif kind == 'A':
                q_bufs[g][...] = jnp.dot(x_v[...], wq_v[g], preferred_element_type=f32).astype(jnp.bfloat16)
            elif kind == 'B':
                for b in range(B):
                    _attention(q_bufs[g], k_v, v_v, o_bufs[g], g, b)
            elif g == 0:
                acc_ref[...] = jnp.dot(o_bufs[g][...], wo_v[g], preferred_element_type=f32)
            elif g < HKV - 1:
                acc_ref[...] += jnp.dot(o_bufs[g][...], wo_v[g], preferred_element_type=f32)
            else:
                for i in range(NOC):
                    cols = pl.ds(i * OC, OC)
                    out_v[:, cols] = (acc_ref[:, cols]
                                      + jnp.dot(o_bufs[g][...], wo_v[g, :, cols], preferred_element_type=f32)
                                      ).astype(out_v.dtype)
                    cout[i].start()
    for cp in cout:
        cp.wait()


@jax.jit
def pallas_standalone__gqa_block_cached__near_ridge_kernel(
    x: jax.Array,
    k_cache: jax.Array,
    v_cache: jax.Array,
    wq: jax.Array,
    wo: jax.Array,
):
    bf16, f32 = jnp.bfloat16, jnp.float32
    out = pl.pallas_call(
        _kernel,
        in_specs=[pl.BlockSpec(memory_space=pl.ANY)] * 5,
        out_specs=pl.BlockSpec(memory_space=pl.ANY),
        out_shape=jax.ShapeDtypeStruct((M, D), bf16),
        scratch_shapes=[
            pltpu.VMEM((M, D), bf16),
            pltpu.VMEM((B, HKV, SK, DH), bf16),
            pltpu.VMEM((B, HKV, SK, DH), bf16),
            pltpu.VMEM((HKV, D, GW), bf16),
            pltpu.VMEM((HKV, GW, D), bf16),
            pltpu.VMEM((M, D), f32),
            pltpu.VMEM((M, D), bf16),
            pltpu.SemaphoreType.DMA((NSEM,)),
        ] + [pltpu.VMEM((M, GW), bf16) for _ in range(2 * HKV)]
          + [pltpu.VMEM((M, GW), f32) for _ in CHUNKED],
        compiler_params=pltpu.CompilerParams(vmem_limit_bytes=100 * 1024 * 1024),
    )(x.reshape(M, D), k_cache, v_cache, wq, wo)
    return out.reshape(B, SQ, D)
```
